```python
import jax
import jax.numpy as jnp

def _softmax(x, axis=-1):
    return jax.nn.softmax(x, axis=axis)
def _gelu(x):
    return jax.nn.gelu(x, approximate=True)
def _silu(x):
    return jax.nn.silu(x)
def _sigmoid(x):
    return jax.nn.sigmoid(x)
def _layernorm(x, axis=-1, eps=1e-5):
    m = jnp.mean(x, axis=axis, keepdims=True)
    v = jnp.var(x, axis=axis, keepdims=True)
    return (x - m) / jnp.sqrt(v + eps)
def _scatter_add(tgt, idx, src, axis=0):
    return tgt.at[idx].add(src)
def _segment_sum(src, seg, n):
    return jax.ops.segment_sum(src, seg, n)
class _Rng:
    def __init__(self, key):
        self._k = key
    def _next(self):
        self._k, sub = jax.random.split(self._k)
        return sub
    def normal(self, shape):
        return jax.random.normal(self._next(), shape, dtype=jnp.bfloat16)
    def randint(self, lo, hi, shape):
        return jax.random.randint(self._next(), shape, lo, hi, dtype=jnp.int32)
    def uniform(self, shape, lo=0.0, hi=1.0):
        return jax.random.uniform(self._next(), shape, jnp.bfloat16, lo, hi)
    def permutation(self, n):
        return jax.random.permutation(self._next(), n)


kernel_name = 'standalone__structured_sparse_n_m__ragged'

def setup_inputs():
    _rng = _Rng(jax.random.key(int.from_bytes(__import__("os").urandom(4), "little")))
    _w = (lambda a: (lambda t: t.astype(jnp.bfloat16) if jnp.issubdtype(t.dtype, jnp.floating) else t)(jnp.asarray(a)))
    B, S, D = 16, 4096, 576
    assert D % 4 == 0, "d_model must be divisible by M=4 for 2:4 sparsity"
    return {
        "x": _w((lambda *s: _rng.normal(s) * 0.05)(B, S, D)),
        "w": _w((lambda *s: _rng.normal(s) * 0.05)(D, D)),
        "b": _w((lambda *s: _rng.normal(s) * 0.05)(D)),
    }

def reference(x, w, b):
    B, S, D = x.shape
    N, M = 2, 4
    G = D // M
    wg = w.reshape(G, M, D)
    mag = jnp.abs(wg)
    order = jnp.argsort(mag, 1)
    thr = jnp.take_along_axis(mag, order[:, M - N:M - N + 1, :], 1)
    mask = (lambda x, dt: x.astype(dt))(mag >= thr, w.dtype)
    wp = (wg * mask).reshape(D, D)
    return jnp.einsum("bsd,df->bsf", x, wp) + b
```

```python
import jax
import jax.numpy as jnp
from jax import lax
import jax.experimental.pallas as pl
import jax.experimental.pallas.tpu as pltpu

BF16, F32, I32 = jnp.bfloat16, jnp.float32, jnp.int32

GROUP = 512
SPAN = 8
X_COLS = 128
O_COLS = 256
FIRST = (1, 1, 2, 4)
PRE = 6
WRITE_FROM = 63
OUT_SPANS = 9
SHARED = (2, 5, 6, 7)


def _prune_packed(u):
    mate = lax.broadcasted_iota(I32, u.shape, 0) ^ 1
    lo = pltpu.bitcast((u << 16) & 0x7FFFFFFF, F32)
    hi = pltpu.bitcast(u & 0x7FFF0000, F32)
    big, small = jnp.maximum(lo, hi), jnp.minimum(lo, hi)
    nbig = jnp.take_along_axis(big, mate, axis=0, mode="promise_in_bounds")
    nsmall = jnp.take_along_axis(small, mate, axis=0, mode="promise_in_bounds")
    thr = jnp.maximum(jnp.minimum(big, nbig), jnp.maximum(small, nsmall))
    return u & (jnp.where(lo < thr, 0, 0xFFFF) | jnp.where(hi < thr, 0, -65536))


class _Rows:
    def __init__(self, bf16=None, f32=None):
        self._bf16, self._f32 = bf16, f32

    def f32(self):
        if self._f32 is None:
            self._f32 = self._bf16.astype(F32)
        return self._f32

    def bf16(self):
        if self._bf16 is None:
            self._bf16 = self._f32.astype(BF16)
        return self._bf16

    def __add__(self, other):
        return _Rows(f32=self.f32() + other.f32())

    def __sub__(self, other):
        return _Rows(f32=self.f32() - other.f32())


def _kernel(x_hbm, w_hbm, b_hbm, o_hbm, xbuf, obuf, wbuf, bbuf, wt, bias_ref, isem, osem, wsem):
    NB, D, S = x_hbm.shape
    F = w_hbm.shape[1]
    H = F // 2
    per_batch = S // GROUP
    NG = NB * per_batch
    NIT = NG // SPAN
    nx, no = GROUP // X_COLS, GROUP // O_COLS
    lg_batch, lg_span = per_batch.bit_length() - 1, SPAN.bit_length() - 1
    first_at = [sum(FIRST[:i]) for i in range(len(FIRST))]
    assert D == F == 576 and sum(FIRST) == SPAN and OUT_SPANS < NIT <= 2 * OUT_SPANS

    def cols(ref, g, j, width):
        start = (g & (per_batch - 1)) * GROUP + j * width
        if not isinstance(g, int):
            start = pl.multiple_of(start, 128)
        return ref.at[g >> lg_batch, :, pl.ds(start, width)]

    def start_reads(g):
        if isinstance(g, int) and g < SPAN:
            sem = NIT + max(i for i, f in enumerate(first_at) if f <= g)
        else:
            sem = g >> lg_span
        for j in range(nx):
            pltpu.make_async_copy(cols(x_hbm, g, j, X_COLS), xbuf.at[g * nx + j], isem.at[sem]).start()

    def wait_reads(g, n, sem):
        filled = xbuf.at[pl.ds(g * nx, n * nx)]
        pltpu.make_async_copy(filled, filled, isem.at[sem]).wait()

    def ring(span):
        if isinstance(span, int):
            return span % OUT_SPANS
        return jnp.where(span >= OUT_SPANS, span - OUT_SPANS, span)

    def writes(g):
        slot = ring(g >> lg_span)
        return [pltpu.make_async_copy(obuf.at[(slot * SPAN + (g & (SPAN - 1))) * no + j],
                                      cols(o_hbm, g, j, O_COLS), osem.at[slot]) for j in range(no)]

    def wait_writes(slot):
        drained = obuf.at[pl.ds(slot * SPAN * no, SPAN * no)]
        pltpu.make_async_copy(drained, drained, osem.at[slot]).wait()

    w_copy = pltpu.make_async_copy(w_hbm, wbuf, wsem.at[0])
    b_copy = pltpu.make_async_copy(b_hbm, bbuf, wsem.at[1])
    w_copy.start()
    b_copy.start()
    for g in range(PRE):
        start_reads(g)

    w_copy.wait()
    words = pltpu.bitcast(wbuf[...], I32)
    pruned = [_prune_packed(words[i:i + 8]) for i in range(0, D // 2, 8)]
    a = pltpu.bitcast(jnp.concatenate(pruned + pruned[32:], axis=0), BF16).T.astype(F32)
    a1, a2 = a[:H], a[H:]
    p, q, c = slice(0, 256), slice(256, 512), slice(512, 640)
    main = {1: a1[:, p] + a2[:, q], 2: a2[:, p] + a2[:, q], 3: a1[:, p], 4: a2[:, q],
            5: a1[:, p] + a1[:, q], 6: a2[:, p] - a1[:, p], 7: a1[:, q] - a2[:, q]}
    rest = {2: a2[:, c], 5: a1[:, c], 6: a2[:, c], 7: a1[:, c]}
    low = lax.broadcasted_iota(I32, (H, 128), 1) < 64
    left = {}
    for j in range(1, 8):
        tiles = {"01": main[j][:, :128], "23": main[j][:, 128:]}
        if j in SHARED:
            tiles["24"] = jnp.where(low, main[j][:, 128:], rest[j])
            tiles["43"] = jnp.where(low, rest[j], main[j][:, 128:])
        for name, tile in tiles.items():
            left[j, name] = len(left)
            wt[left[j, name]] = tile.astype(BF16)
    b_copy.wait()
    bias_ref[...] = jnp.broadcast_to(bbuf[...].reshape(1, F).astype(F32), (128, F)).T

    x_words = xbuf.bitcast(I32)
    w_words = wt.bitcast(I32)

    def mxu_pass(j, name, top, bottom):
        rhs = jnp.concatenate([top.bf16(), bottom.bf16()], axis=0)
        return jnp.dot(pltpu.bitcast(w_words[left[j, name]], BF16), rhs, preferred_element_type=F32)

    def compute_group(g, slot):
        def load(tile, kb):
            i, o = divmod(tile * 128, X_COLS)
            return _Rows(bf16=pltpu.bitcast(x_words[g * nx + i, pl.ds(kb * 32, 32), pl.ds(o, 128)], BF16))

        def store(tile, half, value):
            i, o = divmod(tile * 128, O_COLS)
            obuf[slot * no + i, pl.ds(half * H, H), pl.ds(o, 128)] = value.astype(BF16)

        x = [[load(tile, kb) for kb in range(9)] for tile in range(4)]

        def right(pair, j, kb):
            u, v = x[2 * pair], x[2 * pair + 1]
            if kb == 4:
                return u[8] if j == 2 else v[8] if j == 5 else u[8] + v[8]
            if j == 1:
                return u[kb] + v[kb + 4]
            if j == 2:
                return u[kb]
            if j == 3:
                return v[kb] - v[kb + 4]
            if j == 4:
                return u[kb + 4] - u[kb]
            if j == 5:
                return v[kb + 4]
            return u[kb] + v[kb] if j == 6 else u[kb + 4] + v[kb + 4]

        def product(pair, j):
            head = mxu_pass(j, "01", right(pair, j, 0), right(pair, j, 1))
            if j not in SHARED:
                return head + mxu_pass(j, "23", right(pair, j, 2), right(pair, j, 3))
            if pair == 0:
                return head + mxu_pass(j, "23", right(0, j, 2), right(0, j, 3) - right(1, j, 3))
            return head + mxu_pass(j, "24", right(1, j, 2), right(1, j, 4) - right(0, j, 4))

        shared = {j: mxu_pass(j, "43", right(0, j, 4), right(1, j, 3)) for j in SHARED}
        b1, b2 = bias_ref[0:H], bias_ref[H:F]
        t11, t12 = shared[7] - shared[5] + b1, shared[5] + b1
        t21, t22 = shared[2] + b2, shared[6] - shared[2] + b2
        c11 = []
        for pair in range(2):
            m1, m4 = product(pair, 1), product(pair, 4)
            m3, m5 = product(pair, 3), product(pair, 5)
            store(2 * pair + 1, 0, m3 + m5 + t12)
            c11.append(m1 + m4 + t11 - m5)
            c22 = m1 + t22 + m3
            m2, m6 = product(pair, 2), product(pair, 6)
            store(2 * pair, 1, m4 + t21 + m2)
            store(2 * pair + 1, 1, c22 - m2 + m6)
        for pair in range(2):
            store(2 * pair, 0, c11[pair] + product(pair, 7))

    def body(t, written):
        slot = ring(t)

        @pl.when(t > 0)
        def _():
            wait_reads(t * SPAN, SPAN, t)

        @pl.when(t >= OUT_SPANS)
        def _():
            wait_writes(slot)

        for gi in range(SPAN):
            g = t * SPAN + gi
            for r in range(2):
                ahead = PRE + 2 * gi + r
                more = PRE + 2 * g + r < NG
                if ahead < SPAN:
                    @pl.when(t == 0)
                    def _():
                        start_reads(ahead)
                    more = jnp.logical_and(t > 0, more)

                @pl.when(more)
                def _():
                    start_reads(PRE + 2 * g + r)
            for r in range(2):
                go = jnp.logical_and(g >= WRITE_FROM, written < g)
                copies = writes(written)

                @pl.when(go)
                def _():
                    for copy in copies:
                        copy.start()
                written = written + go.astype(I32)
            if gi in first_at:
                i = first_at.index(gi)

                @pl.when(t == 0)
                def _():
                    wait_reads(gi, FIRST[i], NIT + i)
            compute_group(g, slot * SPAN + gi)
        return written

    lax.fori_loop(0, NIT, body, 0)
    for g in range(min(NG - 1, 2 * (NG - WRITE_FROM)), NG):
        for copy in writes(g):
            copy.start()
    for span in range(NIT - OUT_SPANS, NIT):
        wait_writes(ring(span))


@jax.jit
def pallas_standalone__structured_sparse_n_m__ragged_kernel(
    x: jax.Array,
    w: jax.Array,
    b: jax.Array,
):
    B, S, D = x.shape
    F = w.shape[1]
    spans = B * S // (GROUP * SPAN)
    out = pl.pallas_call(
        _kernel,
        in_specs=[pl.BlockSpec(memory_space=pl.ANY)] * 3,
        out_specs=pl.BlockSpec(memory_space=pl.ANY),
        out_shape=jax.ShapeDtypeStruct((B, F, S), x.dtype),
        scratch_shapes=[
            pltpu.VMEM((B * S // X_COLS, D, X_COLS), x.dtype),
            pltpu.VMEM((OUT_SPANS * SPAN * GROUP // O_COLS, F, O_COLS), x.dtype),
            pltpu.VMEM((D, F), w.dtype),
            pltpu.VMEM((F,), b.dtype),
            pltpu.VMEM((14 + 2 * len(SHARED), F // 2, 128), BF16),
            pltpu.VMEM((F, 128), F32),
            pltpu.SemaphoreType.DMA((spans + len(FIRST),)),
            pltpu.SemaphoreType.DMA((OUT_SPANS,)),
            pltpu.SemaphoreType.DMA((2,)),
        ],
        compiler_params=pltpu.CompilerParams(
            vmem_limit_bytes=127 * 1024 * 1024,
            flags={"XLA_TPU_RESCHEDULE_DMA_DONES": True},
            disable_bounds_checks=True,
            disable_semaphore_checks=True,
        ),
    )(jnp.transpose(x, (0, 2, 1)), w, b)
    return jnp.transpose(out, (0, 2, 1))
```

```python
import jax
import jax.numpy as jnp
from jax import lax
import jax.experimental.pallas as pl
import jax.experimental.pallas.tpu as pltpu

BF16, F32, I32 = jnp.bfloat16, jnp.float32, jnp.int32

GROUP = 512
SPAN = 8
SLOTS = 8
STRIPES = (0, 4, 2, 6, 1, 5, 3, 7)
FIRST = (1, 1, 2, 4)
PRE, PRE_URGENT = 4, 1
W_PIECES = 12
WRITE_FROM = 500
LAST = (4, 2, 2)
OUT_SPANS = 10

LEFT = {
    "d1": "+00-01-20", "d2": "+00-02-10", "d3": "+11-01-12",
    "d4": "+10-11+21", "d5": "+22-02-21", "d6": "+22-12-20",
    "p1": "+01", "p2": "+10", "p3": "+10-01",
    "q1": "+02", "q2": "+20", "q3": "+20-02",
    "r1": "+12", "r2": "+21", "r3": "+12-21",
}


def _prune_packed(u):
    mate = lax.broadcasted_iota(I32, u.shape, 0) ^ 1
    lo = pltpu.bitcast((u << 16) & 0x7FFFFFFF, F32)
    hi = pltpu.bitcast(u & 0x7FFF0000, F32)
    big, small = jnp.maximum(lo, hi), jnp.minimum(lo, hi)
    nbig = jnp.take_along_axis(big, mate, axis=0, mode="promise_in_bounds")
    nsmall = jnp.take_along_axis(small, mate, axis=0, mode="promise_in_bounds")
    thr = jnp.maximum(jnp.minimum(big, nbig), jnp.maximum(small, nsmall))
    return u & (jnp.where(lo < thr, 0, 0xFFFF) | jnp.where(hi < thr, 0, -65536))


def _build_left(w, left_ref):
    words = pltpu.bitcast(w, I32)
    pruned = [_prune_packed(words[r:r + 8]) for r in range(0, words.shape[0], 8)]
    rows = []
    for k in range(3):
        rows += pruned[12 * k:12 * k + 12] + pruned[12 * k + 8:12 * k + 12]
    a = pltpu.bitcast(jnp.concatenate(rows, axis=0), BF16).T.astype(F32)
    low = lax.broadcasted_iota(I32, (96, 128), 1) < 64
    for n, terms in enumerate(LEFT.values()):
        acc = None
        for p in range(0, len(terms), 3):
            i, k = int(terms[p + 1]), int(terms[p + 2])
            block = a[192 * i:192 * i + 192, 256 * k:256 * k + 256]
            acc = block if acc is None else acc + block if terms[p] == "+" else acc - block
        u_ab, u_cc, l_ab, l_cc = acc[:96, :128], acc[:96, 128:], acc[96:, :128], acc[96:, 128:]
        left_ref[3 * n] = jnp.where(low, u_ab, u_ab - l_ab).astype(BF16)
        left_ref[3 * n + 1] = jnp.where(low, l_ab, l_cc - u_cc).astype(BF16)
        left_ref[3 * n + 2] = jnp.where(low, u_cc, l_ab).astype(BF16)


def _tile_pair(load, store, left, bias, tick):
    raw_u = lambda k: [load(3 * k + c, 0) for c in range(3)]
    raw_v = lambda k: [load(3 * k + c, 1) for c in range(3)]
    u = lambda k: [r.astype(F32) for r in raw_u(k)]
    v = lambda k: [r.astype(F32) for r in raw_v(k)]
    add = lambda p, q: [s + t for s, t in zip(p, q)]
    sub = lambda p, q: [s - t for s, t in zip(p, q)]

    def product(name, right):
        n = 3 * list(LEFT).index(name)

        def mxu_pass(tile, top, bottom):
            rhs = jnp.concatenate([top, bottom], axis=0).astype(BF16)
            return jnp.dot(left(n + tile), rhs, preferred_element_type=F32)

        shared = mxu_pass(2, right[2], right[1])
        upper = mxu_pass(0, right[0], right[1]) + shared
        lower = mxu_pass(1, right[0], right[2]) + shared
        tick()
        return jnp.concatenate([upper, lower], axis=0)

    d1 = product("d1", raw_u(0))
    q2 = product("q2", add(v(0), v(2)))
    s0 = add(u(0), v(0))
    t0 = add(s0, v(2))
    q3 = product("q3", t0)
    g = q3 - q2
    e0 = d1 + g
    q1 = product("q1", add(t0, u(2)))
    c0u = e0 + q1 + bias(0)
    c2u = product("d5", raw_u(2)) + (g + q1 + bias(2))
    c0v = product("d2", s0) + (bias(0) - e0)
    p1 = product("p1", add(u(0), u(1)))
    c0u = c0u + p1
    p3 = product("p3", sub(u(0), v(1)))
    c1u = p1 + p3 + bias(1)
    p2 = product("p2", add(v(0), v(1)))
    store(0, c0u, c0v + p3 + p2)
    d4 = product("d4", raw_v(1))
    r2 = product("r2", add(u(1), u(2)))
    c2u = c2u + r2
    s1 = add(u(1), v(1))
    t1 = add(s1, u(2))
    r3 = product("r3", t1)
    h = r2 + r3
    e1 = d4 + h
    c1u = product("d3", s1) + (c1u + e1)
    r1 = product("r1", add(t1, v(2)))
    store(1, c1u, r1 + (p2 + bias(1) - e1))
    c2v = product("d6", raw_v(2)) + (r1 + (q2 + bias(2) - h))
    store(2, c2u, c2v)


def _kernel(x_hbm, w_hbm, b_hbm, o_hbm, xbuf, obuf, wbuf, bbuf, left_ref, bias_ref, isem, osem, wsem):
    D, F = w_hbm.shape
    NB = x_hbm.shape[0] // 9
    first_at = [sum(FIRST[:i]) for i in range(len(FIRST))]
    assert D == F == 576 and x_hbm.shape[-1] == SPAN * GROUP and OUT_SPANS < NB <= 2 * OUT_SPANS

    def stripe(ref, batch, j, col):
        start = col * GROUP if isinstance(col, int) else pl.multiple_of(col * GROUP, GROUP)
        return ref.at[pl.ds(batch * 9, 9), j, :, pl.ds(start, GROUP)]

    def read(batch, col, j, sem):
        return pltpu.make_async_copy(
            stripe(x_hbm, batch, j, col), xbuf.at[batch * SPAN + col, :, j], isem.at[sem])

    def wait_reads(g, n, sem):
        filled = xbuf.at[pl.ds(g, n)]
        pltpu.make_async_copy(filled, filled, isem.at[sem]).wait()

    def first_sem(col):
        return NB + sum(jnp.where(col >= f, 1, 0) for f in first_at[1:])

    def ring(batch):
        return jnp.where(batch >= OUT_SPANS, batch - OUT_SPANS, batch)

    def write(n):
        batch, r = n >> 6, n & 63
        lg_width, col0 = 3, 0
        for i, width in enumerate(LAST):
            here = jnp.logical_and(batch >= NB - 1, r >= 8 * sum(LAST[:i]))
            lg_width = jnp.where(here, width.bit_length() - 1, lg_width)
            col0 = jnp.where(here, sum(LAST[:i]), col0)
        q = r - 8 * col0
        j = q >> lg_width
        col = col0 + q - (j << lg_width)
        valid = jnp.minimum(batch, NB - 1)
        slot = ring(valid)
        copy = pltpu.make_async_copy(
            obuf.at[slot * SPAN + col, :, j], stripe(o_hbm, valid, j, col), osem.at[slot])
        return copy, batch * SPAN + col

    def wait_writes(slot):
        drained = obuf.at[pl.ds(slot * SPAN, SPAN)]
        pltpu.make_async_copy(drained, drained, osem.at[slot]).wait()

    def start_w(i, carry):
        rows = pl.ds(pl.multiple_of(i * (D // W_PIECES), 16), D // W_PIECES)
        pltpu.make_async_copy(w_hbm.at[rows], wbuf.at[rows], wsem.at[0]).start()

    def start_x(priority):
        def start(col, carry):
            for j in STRIPES:
                read(0, col, j, first_sem(col)).start(priority=priority)
        return start

    b_copy = pltpu.make_async_copy(b_hbm, bbuf, wsem.at[1])
    lax.fori_loop(0, W_PIECES, start_w, None)
    b_copy.start()
    lax.fori_loop(0, PRE_URGENT, start_x(0), None)
    lax.fori_loop(PRE_URGENT, PRE, start_x(1), None)
    pltpu.make_async_copy(wbuf, wbuf, wsem.at[0]).wait()
    _build_left(wbuf[...], left_ref)
    b_copy.wait()
    bias_ref[...] = jnp.broadcast_to(bbuf[...].reshape(1, F).astype(F32), (128, F)).T
    left_words = left_ref.bitcast(I32)

    def issue(t, point, written):
        ahead, q = divmod(8 * PRE + 2 * point, 8)
        batch, col = 2 * t + ahead // SPAN, ahead % SPAN
        sem = jnp.where(t == 0, first_sem(col), batch) if ahead < SPAN else batch

        @pl.when(batch < NB)
        def _():
            read(batch, col, STRIPES[q], sem).start(priority=1)
            read(batch, col, STRIPES[q + 1], sem).start(priority=0)

        writing = t * (SPAN * SLOTS) + point >= WRITE_FROM
        for _ in range(2):
            copy, needs = write(written)
            go = jnp.logical_and(writing, needs < t * SPAN + point // SLOTS)
            pl.when(go)(copy.start)
            written = written + go.astype(I32)
        return written

    def body(t, written):
        slot = ring(t)
        pl.when(t > 0)(lambda: wait_reads(t * SPAN, SPAN, t))
        pl.when(t >= OUT_SPANS)(lambda: wait_writes(slot))
        state = {"written": written, "products": 0, "points": 0}

        def tick():
            if state["points"] * 2 * len(LEFT) <= state["products"] * SLOTS:
                state["written"] = issue(t, state["points"], state["written"])
                state["points"] += 1
            state["products"] += 1

        for col in range(SPAN):
            if col in first_at:
                i = first_at.index(col)
                pl.when(t == 0)(lambda: wait_reads(col, FIRST[i], NB + i))
            for half in range(2):
                def load(r, tile):
                    cols = pl.ds(256 * half + 128 * tile, 128)
                    return xbuf[t * SPAN + col, r, :, :, cols].reshape(64, 128)

                def store(i, c_u, c_v):
                    both = jnp.concatenate([c_u, c_v], axis=1).astype(BF16)
                    for r in range(3):
                        obuf[slot * SPAN + col, 3 * i + r, :, :, pl.ds(256 * half, 256)] = (
                            both[64 * r:64 * r + 64].reshape(8, 8, 256))

                _tile_pair(load, store, lambda n: pltpu.bitcast(left_words[n], BF16),
                           lambda i: bias_ref[pl.ds(192 * i, 192)], tick)
        assert state["points"] == SPAN * SLOTS
        return state["written"]

    written = lax.fori_loop(0, NB, body, 0)
    lax.fori_loop(written, NB * 64, lambda n, carry: write(n)[0].start(), None)
    for batch in range(NB - OUT_SPANS, NB):
        wait_writes(batch % OUT_SPANS)


@jax.jit
def pallas_standalone__structured_sparse_n_m__ragged_kernel(
    x: jax.Array,
    w: jax.Array,
    b: jax.Array,
):
    B, S, D = x.shape
    F = w.shape[1]
    striped = (B * D // 64, 8, 8, S)
    out = pl.pallas_call(
        _kernel,
        in_specs=[pl.BlockSpec(memory_space=pl.ANY)] * 3,
        out_specs=pl.BlockSpec(memory_space=pl.ANY),
        out_shape=jax.ShapeDtypeStruct(striped, x.dtype),
        scratch_shapes=[
            pltpu.VMEM((B * SPAN, D // 64, 8, 8, GROUP), x.dtype),
            pltpu.VMEM((OUT_SPANS * SPAN, F // 64, 8, 8, GROUP), x.dtype),
            pltpu.VMEM((D, F), w.dtype),
            pltpu.VMEM((F,), b.dtype),
            pltpu.VMEM((3 * len(LEFT), 96, 128), BF16),
            pltpu.VMEM((F, 128), F32),
            pltpu.SemaphoreType.DMA((B + len(FIRST),)),
            pltpu.SemaphoreType.DMA((OUT_SPANS,)),
            pltpu.SemaphoreType.DMA((2,)),
        ],
        compiler_params=pltpu.CompilerParams(
            vmem_limit_bytes=127 * 1024 * 1024,
            flags={"XLA_TPU_RESCHEDULE_DMA_DONES": True},
            disable_bounds_checks=True,
            disable_semaphore_checks=True,
        ),
    )(jnp.transpose(x, (0, 2, 1)).reshape(striped), w, b)
    return jnp.transpose(out.reshape(B, F, S), (0, 2, 1))
```

```python
import jax
import jax.numpy as jnp
from jax import lax
import jax.experimental.pallas as pl
import jax.experimental.pallas.tpu as pltpu

BF16, F32, I32 = jnp.bfloat16, jnp.float32, jnp.int32

X_COLS = 512
O_COLS = 1024
POINTS = 128
FIRST = (1, 1, 2, 4)
PRE = 4
W_PIECES = 12
WRITE_FROM = 1012
WRITE_LEAD = 4
OUT_PAIRS = 5

LEFT = {
    "d1": "+00-01-20", "d2": "+00-02-10", "d3": "+11-01-12",
    "d4": "+10-11+21", "d5": "+22-02-21", "d6": "+22-12-20",
    "p1": "+01", "p2": "+10", "p3": "+10-01",
    "q1": "+02", "q2": "+20", "q3": "+20-02",
    "r1": "+12", "r2": "+21", "r3": "+12-21",
}


def _prune_packed(u):
    mate = lax.broadcasted_iota(I32, u.shape, 0) ^ 1
    lo = pltpu.bitcast((u << 16) & 0x7FFFFFFF, F32)
    hi = pltpu.bitcast(u & 0x7FFF0000, F32)
    big, small = jnp.maximum(lo, hi), jnp.minimum(lo, hi)
    nbig = jnp.take_along_axis(big, mate, axis=0, mode="promise_in_bounds")
    nsmall = jnp.take_along_axis(small, mate, axis=0, mode="promise_in_bounds")
    thr = jnp.maximum(jnp.minimum(big, nbig), jnp.maximum(small, nsmall))
    return u & (jnp.where(lo < thr, 0, 0xFFFF) | jnp.where(hi < thr, 0, -65536))


def _build_left(w, left_ref):
    words = pltpu.bitcast(w, I32)
    pruned = [_prune_packed(words[r:r + 8]) for r in range(0, words.shape[0], 8)]
    rows = []
    for k in range(3):
        rows += pruned[12 * k:12 * k + 12] + pruned[12 * k + 8:12 * k + 12]
    a = pltpu.bitcast(jnp.concatenate(rows, axis=0), BF16).T.astype(F32)
    low = lax.broadcasted_iota(I32, (96, 128), 1) < 64
    tiles = {}
    for i in range(3):
        for k in range(3):
            block = a[192 * i:192 * i + 192, 256 * k:256 * k + 256]
            u_ab, u_cc, l_ab, l_cc = block[:96, :128], block[:96, 128:], block[96:, :128], block[96:, 128:]
            tiles[f"{i}{k}"] = (jnp.where(low, u_ab, u_ab - l_ab), jnp.where(low, l_ab, l_cc - u_cc),
                                jnp.where(low, u_cc, l_ab))
    for n, terms in enumerate(LEFT.values()):
        for m in range(3):
            acc = tiles[terms[1:3]][m]
            for p in range(3, len(terms), 3):
                term = tiles[terms[p + 1:p + 3]][m]
                acc = acc + term if terms[p] == "+" else acc - term
            left_ref[3 * n + m] = acc.astype(BF16)


def _tile_pair(load, store, left, bias, tick):
    raw_u = lambda k: [load(3 * k + c, 0) for c in range(3)]
    raw_v = lambda k: [load(3 * k + c, 1) for c in range(3)]
    u = lambda k: [r.astype(F32) for r in raw_u(k)]
    v = lambda k: [r.astype(F32) for r in raw_v(k)]
    add = lambda p, q: [s + t for s, t in zip(p, q)]
    sub = lambda p, q: [s - t for s, t in zip(p, q)]

    def product(name, right):
        n = 3 * list(LEFT).index(name)

        def mxu_pass(tile, top, bottom):
            rhs = jnp.concatenate([top, bottom], axis=0).astype(BF16)
            return jnp.dot(left(n + tile), rhs, preferred_element_type=F32)

        lower = mxu_pass(1, right[0], right[2])
        shared = mxu_pass(2, right[2], right[1])
        upper = mxu_pass(0, right[0], right[1])
        result = jnp.concatenate([upper + shared, lower + shared], axis=0)
        tick()
        return result

    d1 = product("d1", raw_u(0))
    q2 = product("q2", add(v(0), v(2)))
    c2v = bias(2) + q2
    s0 = add(u(0), v(0))
    t0 = add(s0, v(2))
    q1 = product("q1", add(t0, u(2)))
    d2 = product("d2", s0)
    c0u = bias(0) + q1
    g = product("q3", t0) - q2
    e0 = d1 + g
    c0u = c0u + e0
    p3 = product("p3", sub(u(0), v(1)))
    p1 = product("p1", add(u(0), u(1)))
    c0u = c0u + p1
    d5 = product("d5", raw_u(2))
    c1u = bias(1) + p1 + p3
    d4 = product("d4", raw_v(1))
    c0v = bias(0) + d2 - e0 + p3
    p2 = product("p2", add(v(0), v(1)))
    store(0, c0u, c0v + p2)
    r2 = product("r2", add(u(1), u(2)))
    c1v = bias(1) + p2
    c2u = bias(2) + d5 + g + q1 + r2
    s1 = add(u(1), v(1))
    t1 = add(s1, u(2))
    r1 = product("r1", add(t1, v(2)))
    c1v = c1v + r1
    d6 = product("d6", raw_v(2))
    c1u = c1u + product("d3", s1)
    h = r2 + product("r3", t1)
    e1 = d4 + h
    store(1, c1u + e1, c1v - e1)
    store(2, c2u, c2v + d6 + r1 - h)


def _kernel(x_hbm, w_hbm, b_hbm, o_hbm, xbuf, even, odd, wbuf, bbuf, left_ref, bias_ref, isem, osem, wsem):
    D, F = w_hbm.shape
    NB = x_hbm.shape[0] // 9
    cols = xbuf.shape[0]
    first_at = [sum(FIRST[:i]) for i in range(len(FIRST))]
    assert D == F == 576 and NB == 16 and cols == 8 and even.shape[0] == 4 and PRE == first_at[-1]

    def columns(col, width):
        return pl.ds(col * width if isinstance(col, int) else pl.multiple_of(col * width, width), width)

    def read(run, n, j, col, sem):
        return pltpu.make_async_copy(x_hbm.at[pl.ds(run, n), j, :, columns(col, X_COLS)],
                                     xbuf.at[col, pl.ds(run, n), j], isem.at[sem])

    def wait_reads(batch, col, n, sem):
        filled = xbuf.at[pl.ds(col, n), pl.ds(9 * batch, 9)]
        pltpu.make_async_copy(filled, filled, isem.at[sem]).wait()

    def ring(batch):
        if isinstance(batch, int):
            return batch % (2 * OUT_PAIRS)
        return jnp.where(batch >= 2 * OUT_PAIRS, batch - 2 * OUT_PAIRS, batch)

    def write(pair, h, j, col):
        run = 9 * pair
        for i, buf in enumerate((odd, even) if h else (even, odd)):
            n = buf.shape[2]
            pltpu.make_async_copy(buf.at[col, ring(2 * pair) + i, :, j],
                                  o_hbm.at[pl.ds(run, n), h, j, :, columns(col, O_COLS)], osem.at[pair]).start()
            run += n

    def wait_writes(pair):
        for buf in (even, odd):
            drained = buf.at[:, pl.ds(ring(2 * pair), 2)]
            pltpu.make_async_copy(drained, drained, osem.at[pair]).wait()

    def by_row(q):
        return q >> 5, (q >> 2) & 7, q & 3

    def by_column(q):
        return (q >> 2) & 1, ((q & 3) << 1) | ((q >> 3) & 1), q >> 4

    def start_w(i, carry):
        rows = pl.ds(pl.multiple_of(i * (D // W_PIECES), 16), D // W_PIECES)
        pltpu.make_async_copy(w_hbm.at[rows], wbuf.at[rows], wsem.at[0]).start(priority=1)

    def start_x(col, carry):
        sem = NB + sum(jnp.where(col >= f, 1, 0) for f in first_at[1:])
        for j in range(8):
            read(0, 9, j, col, sem).start(priority=1)

    b_copy = pltpu.make_async_copy(b_hbm, bbuf, wsem.at[1])
    lax.fori_loop(0, W_PIECES, start_w, None)
    b_copy.start(priority=1)
    lax.fori_loop(0, PRE, start_x, None)
    pltpu.make_async_copy(wbuf, wbuf, wsem.at[0]).wait()
    _build_left(wbuf[...], left_ref)
    b_copy.wait()
    bias_ref[...] = jnp.broadcast_to(bbuf[...].reshape(1, F).astype(F32), (128, F)).T
    left_words = left_ref.bitcast(I32)

    def issue(t, point):
        ahead, q = divmod(8 * PRE + point, 64)
        batch = 2 * t + ahead
        j, col, sem = q >> 3, q & 7, batch
        if ahead == 0:
            j = jnp.where(t == 0, (q >> 2) & 7, j)
            col = jnp.where(t == 0, PRE + (q & 3), col)
            sem = jnp.where(t == 0, NB + len(FIRST) - 1, sem)

        @pl.when(batch < NB)
        def _():
            read(9 * batch, 8, j, col, sem).start(priority=1)
            read(9 * batch + 8, 1, j, col, sem).start(priority=0)

        if point % 2:
            return
        slot = point // 2
        t_first, first_slot = divmod(WRITE_FROM // 2, 64)
        if slot == first_slot:
            @pl.when(t == t_first)
            def _():
                for q in range(WRITE_LEAD):
                    write(0, *by_row(q))
        carry, q = divmod(slot - first_slot + WRITE_LEAD, 64)
        pair = t - t_first + carry
        steady = jnp.logical_and(t >= t_first + (slot < first_slot), pair < NB // 2 - 2)
        pl.when(steady)(lambda: write(pair, *by_row(q)))
        pl.when(t == NB - 2)(lambda: write(NB // 2 - 2, *by_row(slot)))
        if slot >= 16:
            pl.when(t == NB - 1)(lambda: write(NB // 2 - 1, *by_column(slot - 16)))

    def body(t, carry):
        pl.when(t > 0)(lambda: wait_reads(t, 0, cols, t))
        pl.when(jnp.logical_and(t >= 2 * OUT_PAIRS, (t & 1) == 0))(lambda: wait_writes((t >> 1) - OUT_PAIRS))
        slot = ring(t)
        products, points = [0], [0]

        def tick():
            if points[0] * 2 * cols * len(LEFT) <= products[0] * POINTS:
                issue(t, points[0])
                points[0] += 1
            products[0] += 1

        for col in range(cols):
            if col in first_at:
                i = first_at.index(col)
                pl.when(t == 0)(lambda: wait_reads(0, col, FIRST[i], NB + i))
            for half in range(2):
                def load(r, tile):
                    return xbuf[col, 9 * t + r, :, :, pl.ds(256 * half + 128 * tile, 128)].reshape(64, 128)

                def store(i, c_u, c_v):
                    both = jnp.concatenate([c_u, c_v], axis=1).astype(BF16)
                    for r in range(3 * i, 3 * i + 3):
                        (even, odd)[r % 2][col // 2, slot, r // 2, :, :, pl.ds(512 * (col % 2) + 256 * half, 256)] = (
                            both[64 * (r % 3):64 * (r % 3) + 64].reshape(8, 8, 256))

                _tile_pair(load, store, lambda n: pltpu.bitcast(left_words[n], BF16),
                           lambda i: bias_ref[pl.ds(192 * i, 192)], tick)
        assert points[0] == POINTS

    lax.fori_loop(0, NB, body, None)
    for q in range(48, 64):
        write(NB // 2 - 1, *by_column(q))
    for pair in range(NB // 2 - OUT_PAIRS, NB // 2):
        wait_writes(pair)


@jax.jit
def pallas_standalone__structured_sparse_n_m__ragged_kernel(
    x: jax.Array,
    w: jax.Array,
    b: jax.Array,
):
    B, S, D = x.shape
    F = w.shape[1]
    out = pl.pallas_call(
        _kernel,
        in_specs=[pl.BlockSpec(memory_space=pl.ANY)] * 3,
        out_specs=pl.BlockSpec(memory_space=pl.ANY),
        out_shape=jax.ShapeDtypeStruct((B * F // 128, 2, 8, 8, S), x.dtype),
        scratch_shapes=[
            pltpu.VMEM((S // X_COLS, B * D // 64, 8, 8, X_COLS), x.dtype),
            pltpu.VMEM((S // O_COLS, 2 * OUT_PAIRS, 5, 8, 8, O_COLS), x.dtype),
            pltpu.VMEM((S // O_COLS, 2 * OUT_PAIRS, 4, 8, 8, O_COLS), x.dtype),
            pltpu.VMEM((D, F), w.dtype),
            pltpu.VMEM((F,), b.dtype),
            pltpu.VMEM((3 * len(LEFT), 96, 128), BF16),
            pltpu.VMEM((F, 128), F32),
            pltpu.SemaphoreType.DMA((B + len(FIRST),)),
            pltpu.SemaphoreType.DMA((B // 2,)),
            pltpu.SemaphoreType.DMA((2,)),
        ],
        compiler_params=pltpu.CompilerParams(
            vmem_limit_bytes=127 * 1024 * 1024,
            flags={"XLA_TPU_RESCHEDULE_DMA_DONES": True},
            disable_bounds_checks=True,
            disable_semaphore_checks=True,
        ),
    )(jnp.transpose(x, (0, 2, 1)).reshape(B * D // 64, 8, 8, S), w, b)
    return jnp.transpose(out.reshape(B, F, S), (0, 2, 1))
```

```python
import jax
import jax.numpy as jnp
from jax import lax
import jax.experimental.pallas as pl
import jax.experimental.pallas.tpu as pltpu

BF16, F32, I32 = jnp.bfloat16, jnp.float32, jnp.int32

X_COLS = 512
O_COLS = 1024
POINTS = 128
FIRST = (1, 1, 2, 4)
PRE = 4
WRITE_FROM = 1012
WRITE_LEAD = 4
OUT_PAIRS = 5

LEFT = {
    "d1": "+00-01-20", "d2": "+00-02-10", "d3": "+11-01-12",
    "d4": "+10-11+21", "d5": "+22-02-21", "d6": "+22-12-20",
    "p1": "+01", "p2": "+10", "p3": "+10-01",
    "q1": "+02", "q2": "+20", "q3": "+20-02",
    "r1": "+12", "r2": "+21", "r3": "+12-21",
}


def _prune_packed(u):
    mate = lax.broadcasted_iota(I32, u.shape, 0) ^ 1
    lo = pltpu.bitcast((u << 16) & 0x7FFFFFFF, F32)
    hi = pltpu.bitcast(u & 0x7FFF0000, F32)
    big, small = jnp.maximum(lo, hi), jnp.minimum(lo, hi)
    nbig = jnp.take_along_axis(big, mate, axis=0, mode="promise_in_bounds")
    nsmall = jnp.take_along_axis(small, mate, axis=0, mode="promise_in_bounds")
    thr = jnp.maximum(jnp.minimum(big, nbig), jnp.maximum(small, nsmall))
    return u & (jnp.where(lo < thr, 0, 0xFFFF) | jnp.where(hi < thr, 0, -65536))


def _build_left(w, left_ref):
    words = pltpu.bitcast(w, I32)
    pruned = [_prune_packed(words[r:r + 8]) for r in range(0, words.shape[0], 8)]
    rows = []
    for k in range(3):
        rows += pruned[12 * k:12 * k + 12] + pruned[12 * k + 8:12 * k + 12]
    a = pltpu.bitcast(jnp.concatenate(rows, axis=0), BF16).T.astype(F32)
    low = lax.broadcasted_iota(I32, (96, 128), 1) < 64
    tiles = {}
    for i in range(3):
        for k in range(3):
            block = a[192 * i:192 * i + 192, 256 * k:256 * k + 256]
            u_ab, u_cc, l_ab, l_cc = block[:96, :128], block[:96, 128:], block[96:, :128], block[96:, 128:]
            tiles[f"{i}{k}"] = (jnp.where(low, u_ab, u_ab - l_ab), jnp.where(low, l_ab, l_cc - u_cc),
                                jnp.where(low, u_cc, l_ab))
    for n, terms in enumerate(LEFT.values()):
        for m in range(3):
            acc = tiles[terms[1:3]][m]
            for p in range(3, len(terms), 3):
                term = tiles[terms[p + 1:p + 3]][m]
                acc = acc + term if terms[p] == "+" else acc - term
            left_ref[3 * n + m] = acc.astype(BF16)


def _tile_pair(load, store, left, bias, tick):
    raw_u = lambda k: [load(3 * k + c, 0) for c in range(3)]
    raw_v = lambda k: [load(3 * k + c, 1) for c in range(3)]
    u = lambda k: [r.astype(F32) for r in raw_u(k)]
    v = lambda k: [r.astype(F32) for r in raw_v(k)]
    add = lambda p, q: [s + t for s, t in zip(p, q)]
    sub = lambda p, q: [s - t for s, t in zip(p, q)]

    def product(name, right):
        n = 3 * list(LEFT).index(name)

        def mxu_pass(tile, top, bottom):
            rhs = jnp.concatenate([top, bottom], axis=0).astype(BF16)
            return jnp.dot(left(n + tile), rhs, preferred_element_type=F32)

        lower = mxu_pass(1, right[0], right[2])
        shared = mxu_pass(2, right[2], right[1])
        upper = mxu_pass(0, right[0], right[1])
        result = jnp.concatenate([upper + shared, lower + shared], axis=0)
        tick()
        return result

    d1 = product("d1", raw_u(0))
    q2 = product("q2", add(v(0), v(2)))
    c2v = bias(2) + q2
    s0 = add(u(0), v(0))
    t0 = add(s0, v(2))
    q1 = product("q1", add(t0, u(2)))
    d2 = product("d2", s0)
    c0u = bias(0) + q1
    g = product("q3", t0) - q2
    e0 = d1 + g
    c0u = c0u + e0
    p3 = product("p3", sub(u(0), v(1)))
    p1 = product("p1", add(u(0), u(1)))
    c0u = c0u + p1
    d5 = product("d5", raw_u(2))
    c1u = bias(1) + p1 + p3
    d4 = product("d4", raw_v(1))
    c0v = bias(0) + d2 - e0 + p3
    p2 = product("p2", add(v(0), v(1)))
    store(0, c0u, c0v + p2)
    r2 = product("r2", add(u(1), u(2)))
    c1v = bias(1) + p2
    c2u = bias(2) + d5 + g + q1 + r2
    s1 = add(u(1), v(1))
    t1 = add(s1, u(2))
    r1 = product("r1", add(t1, v(2)))
    c1v = c1v + r1
    d6 = product("d6", raw_v(2))
    c1u = c1u + product("d3", s1)
    h = r2 + product("r3", t1)
    e1 = d4 + h
    store(1, c1u + e1, c1v - e1)
    store(2, c2u, c2v + d6 + r1 - h)


def _kernel(x_hbm, w_hbm, b_hbm, o_hbm, xbuf, even, odd, wbuf, bbuf, left_ref, bias_ref, isem, osem, wsem):
    D, F = w_hbm.shape
    NB = x_hbm.shape[0] // 9
    cols = xbuf.shape[0]
    first_at = [sum(FIRST[:i]) for i in range(len(FIRST))]
    assert D == F == 576 and NB == 16 and cols == 8 and even.shape[0] == 4 and PRE == first_at[-1]

    def columns(col, width):
        return pl.ds(col * width if isinstance(col, int) else pl.multiple_of(col * width, width), width)

    def read(run, n, j, col, sem):
        return pltpu.make_async_copy(x_hbm.at[pl.ds(run, n), j, :, columns(col, X_COLS)],
                                     xbuf.at[col, pl.ds(run, n), j], isem.at[sem])

    def wait_reads(batch, col, n, sem):
        filled = xbuf.at[pl.ds(col, n), pl.ds(9 * batch, 9)]
        pltpu.make_async_copy(filled, filled, isem.at[sem]).wait()

    def ring(batch):
        if isinstance(batch, int):
            return batch % (2 * OUT_PAIRS)
        return jnp.where(batch >= 2 * OUT_PAIRS, batch - 2 * OUT_PAIRS, batch)

    def write(pair, h, j, col):
        run = 9 * pair
        for i, buf in enumerate((odd, even) if h else (even, odd)):
            n = buf.shape[2]
            pltpu.make_async_copy(buf.at[col, ring(2 * pair) + i, :, j],
                                  o_hbm.at[pl.ds(run, n), h, j, :, columns(col, O_COLS)], osem.at[pair]).start()
            run += n

    def wait_writes(pair):
        filled = o_hbm.at[pl.ds(9 * pair, 9)]
        pltpu.make_async_copy(filled, filled, osem.at[pair]).wait()

    def by_row(q):
        return q >> 5, (q >> 2) & 7, q & 3

    def by_column(q):
        return (q >> 2) & 1, ((q & 3) << 1) | ((q >> 3) & 1), q >> 4

    def start_x(col, carry):
        sem = NB + sum(jnp.where(col >= f, 1, 0) for f in first_at[1:])
        for j in range(8):
            read(0, 9, j, col, sem).start(priority=1)

    w_copy = pltpu.make_async_copy(w_hbm, wbuf, wsem.at[0])
    b_copy = pltpu.make_async_copy(b_hbm, bbuf, wsem.at[1])
    w_copy.start(priority=1)
    b_copy.start(priority=1)
    lax.fori_loop(0, PRE, start_x, None)
    w_copy.wait()
    _build_left(wbuf[...], left_ref)
    b_copy.wait()
    bias_ref[...] = jnp.broadcast_to(bbuf[...].reshape(1, F).astype(F32), (128, F)).T
    left_words = left_ref.bitcast(I32)

    def issue(t, point):
        ahead, q = divmod(8 * PRE + point, 64)
        batch = 2 * t + ahead
        j, col, sem = q >> 3, q & 7, batch
        if ahead == 0:
            j = jnp.where(t == 0, (q >> 2) & 7, j)
            col = jnp.where(t == 0, PRE + (q & 3), col)
            sem = jnp.where(t == 0, NB + len(FIRST) - 1, sem)

        @pl.when(batch < NB)
        def _():
            read(9 * batch, 8, j, col, sem).start(priority=1)
            read(9 * batch + 8, 1, j, col, sem).start(priority=0)

        if point % 2:
            return
        slot = point // 2
        t_first, first_slot = divmod(WRITE_FROM // 2, 64)
        if slot == first_slot:
            @pl.when(t == t_first)
            def _():
                for q in range(WRITE_LEAD):
                    write(0, *by_row(q))
        carry, q = divmod(slot - first_slot + WRITE_LEAD, 64)
        pair = t - t_first + carry
        steady = jnp.logical_and(t >= t_first + (slot < first_slot), pair < NB // 2 - 2)
        pl.when(steady)(lambda: write(pair, *by_row(q)))
        pl.when(t == NB - 2)(lambda: write(NB // 2 - 2, *by_row(slot)))
        if slot >= 16:
            pl.when(t == NB - 1)(lambda: write(NB // 2 - 1, *by_column(slot - 16)))

    def body(t, carry):
        pl.when(t > 0)(lambda: wait_reads(t, 0, cols, t))
        pl.when(jnp.logical_and(t >= 2 * OUT_PAIRS, (t & 1) == 0))(lambda: wait_writes((t >> 1) - OUT_PAIRS))
        slot = ring(t)
        products, points = [0], [0]

        def tick():
            if points[0] * 2 * cols * len(LEFT) <= products[0] * POINTS:
                issue(t, points[0])
                points[0] += 1
            products[0] += 1

        for col in range(cols):
            if col in first_at:
                i = first_at.index(col)
                pl.when(t == 0)(lambda: wait_reads(0, col, FIRST[i], NB + i))
            for half in range(2):
                def load(r, tile):
                    return xbuf[col, 9 * t + r, :, :, pl.ds(256 * half + 128 * tile, 128)].reshape(64, 128)

                def store(i, c_u, c_v):
                    both = jnp.concatenate([c_u, c_v], axis=1).astype(BF16)
                    for r in range(3 * i, 3 * i + 3):
                        (even, odd)[r % 2][col // 2, slot, r // 2, :, :, pl.ds(512 * (col % 2) + 256 * half, 256)] = (
                            both[64 * (r % 3):64 * (r % 3) + 64].reshape(8, 8, 256))

                _tile_pair(load, store, lambda n: pltpu.bitcast(left_words[n], BF16),
                           lambda i: bias_ref[pl.ds(192 * i, 192)], tick)
        assert points[0] == POINTS

    lax.fori_loop(0, NB, body, None)
    for q in range(48, 64):
        write(NB // 2 - 1, *by_column(q))
    for pair in range(NB // 2 - OUT_PAIRS, NB // 2):
        wait_writes(pair)


@jax.jit
def pallas_standalone__structured_sparse_n_m__ragged_kernel(
    x: jax.Array,
    w: jax.Array,
    b: jax.Array,
):
    B, S, D = x.shape
    F = w.shape[1]
    out = pl.pallas_call(
        _kernel,
        in_specs=[pl.BlockSpec(memory_space=pl.ANY)] * 3,
        out_specs=pl.BlockSpec(memory_space=pl.ANY),
        out_shape=jax.ShapeDtypeStruct((B * F // 128, 2, 8, 8, S), x.dtype),
        scratch_shapes=[
            pltpu.VMEM((S // X_COLS, B * D // 64, 8, 8, X_COLS), x.dtype),
            pltpu.VMEM((S // O_COLS, 2 * OUT_PAIRS, 5, 8, 8, O_COLS), x.dtype),
            pltpu.VMEM((S // O_COLS, 2 * OUT_PAIRS, 4, 8, 8, O_COLS), x.dtype),
            pltpu.VMEM((D, F), w.dtype),
            pltpu.VMEM((F,), b.dtype),
            pltpu.VMEM((3 * len(LEFT), 96, 128), BF16),
            pltpu.VMEM((F, 128), F32),
            pltpu.SemaphoreType.DMA((B + len(FIRST),)),
            pltpu.SemaphoreType.DMA((B // 2,)),
            pltpu.SemaphoreType.DMA((2,)),
        ],
        compiler_params=pltpu.CompilerParams(
            vmem_limit_bytes=127 * 1024 * 1024,
            flags={"XLA_TPU_RESCHEDULE_DMA_DONES": True},
            disable_bounds_checks=True,
            disable_semaphore_checks=True,
        ),
    )(jnp.transpose(x, (0, 2, 1)).reshape(B * D // 64, 8, 8, S), w, b)
    return jnp.transpose(out.reshape(B, F, S), (0, 2, 1))
```
